```python
import os as _os
_os.environ.setdefault('JAX_PLATFORMS', 'cpu')
import jax
import jax.numpy as jnp

def _softmax(x, axis=-1):
    return jax.nn.softmax(x, axis=axis)

def _gelu(x):
    return jax.nn.gelu(x, approximate=True)

def _silu(x):
    return jax.nn.silu(x)

def _sigmoid(x):
    return jax.nn.sigmoid(x)

def _layernorm(x, axis=-1, eps=1e-05):
    m = jnp.mean(x, axis=axis, keepdims=True)
    v = jnp.var(x, axis=axis, keepdims=True)
    return (x - m) / jnp.sqrt(v + eps)

def _scatter_add(tgt, idx, src, axis=0):
    return tgt.at[idx].add(src)

def _segment_sum(src, seg, n):
    return jax.ops.segment_sum(src, seg, n)

class _Rng:

    def __init__(self, key):
        self._k = key

    def _next(self):
        self._k, sub = jax.random.split(self._k)
        return sub

    def normal(self, shape):
        return jax.random.normal(self._next(), shape, dtype=jnp.bfloat16)

    def randint(self, lo, hi, shape):
        return jax.random.randint(self._next(), shape, lo, hi, dtype=jnp.int32)

    def uniform(self, shape, lo=0.0, hi=1.0):
        return jax.random.uniform(self._next(), shape, jnp.bfloat16, lo, hi)

    def permutation(self, n):
        return jax.random.permutation(self._next(), n)
kernel_name = 'adaLN_cond__sliding_local_dilated__mixer_channel_mlp__prompt'

def setup_inputs():
    _rng = _Rng(jax.random.key(int.from_bytes(__import__("os").urandom(4), "little")))
    _w = lambda a: (lambda t: t.astype(jnp.bfloat16) if jnp.issubdtype(t.dtype, jnp.floating) else t)(jnp.asarray(a))

    def _A_setup():
        B, S, D = (1, 2048, 512)
        return {'x': _w((lambda *s: _rng.normal(s) * 0.05)(B, S, D)), 'wqkv': _w((lambda *s: _rng.normal(s) * 0.05)(D, 3 * D)), 'wo': _w((lambda *s: _rng.normal(s) * 0.05)(D, D))}
    _A_in = _A_setup()

    def _B_setup():
        B, S, D, F = (1, 2048, 512, 1792)
        return {'x': _w((lambda *s: _rng.normal(s) * 0.05)(B, S, D)), 'w1': _w((lambda *s: _rng.normal(s) * 0.8)(D, F) * D ** (-0.5)), 'b1': _w((lambda *s: _rng.normal(s) * 0.8)(F)), 'w2': _w((lambda *s: _rng.normal(s) * 0.8)(F, D) * F ** (-0.5)), 'b2': _w((lambda *s: _rng.normal(s) * 0.4)(D))}
    _B_in = _B_setup()
    return {'A_x': _A_in['x'], 'A_wqkv': _A_in['wqkv'], 'A_wo': _A_in['wo'], 'B_x': _B_in['x'], 'B_w1': _B_in['w1'], 'B_b1': _B_in['b1'], 'B_w2': _B_in['w2'], 'B_b2': _B_in['b2'], 'c': _w((lambda *s: _rng.normal(s) * 0.05)(1, 512) * 8.0), 'w_mod': _w((lambda *s: _rng.normal(s) * 0.05)(512, 6 * 512) * 512 ** (-0.5) * 8.0)}

def reference(A_x, A_wqkv, A_wo, B_x, B_w1, B_b1, B_w2, B_b2, c, w_mod):

    def _A_ref(x, wqkv, wo):
        B, S, D = x.shape
        H = 32
        Dh = D // H
        W, dil = (8, 2)
        qkv = (lambda x, *d: x.transpose(*d))((x @ wqkv).reshape(B, S, 3, H, Dh), 2, 0, 3, 1, 4)
        q, k, v = (qkv[0], qkv[1], qkv[2])
        scale = Dh ** (-0.5)
        pos = jnp.arange(S)
        off = jnp.arange(W) * dil
        idx = pos[:, None] - off[None, :]
        mask = idx >= 0
        idx_c = jnp.where(mask, idx, 0).reshape(-1)
        kg = k[:, :, idx_c, :].reshape(B, H, S, W, Dh)
        vg = v[:, :, idx_c, :].reshape(B, H, S, W, Dh)
        logits = jnp.einsum('bhsd,bhswd->bhsw', q, kg) * scale
        logits = jnp.where(mask[None, None, :, :], logits, -1000000000.0)
        attn = _softmax(logits, axis=-1)
        o = jnp.einsum('bhsw,bhswd->bhsd', attn, vg)
        return (lambda x, *d: x.transpose(*d))(o, 0, 2, 1, 3).reshape(B, S, D) @ wo

    def _B_ref(x, w1, b1, w2, b2):
        y = _layernorm(x, axis=-1)
        h = _gelu(jnp.einsum('bsd,df->bsf', y, w1) + b1)
        return jnp.einsum('bsf,fd->bsd', h, w2) + b2
    x = A_x
    mod = (_silu(c) @ w_mod).reshape(c.shape[0], 6, 1, -1)
    sa, ca, ga, sb, cb, gb = (mod[:, 0].copy(), mod[:, 1].copy(), mod[:, 2].copy(), mod[:, 3].copy(), mod[:, 4].copy(), mod[:, 5].copy())
    h = _layernorm(x, axis=-1) * (1 + ca) + sa
    x = x + ga * _A_ref(h, A_wqkv, A_wo)
    h = _layernorm(x, axis=-1) * (1 + cb) + sb
    x = x + gb * _B_ref(h, B_w1, B_b1, B_w2, B_b2)
    return x
```

```python
import functools
import heapq

import jax
import jax.experimental.pallas as pl
import jax.experimental.pallas.tpu as pltpu
import jax.numpy as jnp
import numpy as np
from jax import lax

S, D, F, H, DH, W = 2048, 512, 1792, 32, 16, 8
EPS = 1e-5
LOG2E = 1.4426950408889634
C0 = 0.7978845608028654
ALPHA = (C0 * 0.044715) ** (1.0 / 3.0)
KAPPA = C0 / ALPHA

f32, bf16, i32 = jnp.float32, jnp.bfloat16, jnp.int32
T = 256
TH = T // 2
NT = S // T
NB = D // 128
FH = F // 256
HALO = 16
PITCH = T + HALO + 8
HEAD_PITCH = DH + 9
TILE_PITCH = 128 + 16
NESTED_PITCH = 64 + 16

SQUARE = (0, 2, 0, 2)
UP = [(0, 2, n, min(n + 2, FH)) for n in range(0, FH, 2)]
DOWN = [(k, min(k + 2, FH), 0, 2) for k in range(0, FH, 2)]
ORDER = (1, 3, 4, 2, 0, 6, 5)
PLAIN = (1, 4)
SUMS = (0, 2, 3, 5, 6)

TIMING = dict(
    after_matmul=310, key_lead=230, act_lead=220, weight_lead=420, permute_lead=600, wq_lead=350,
    attn=(0, 2760, 4900, 0.4, 470), ln1=(5804, 6304, 630), ln2=(7034, 7834, 350),
    fill_ln1=((610, 640, 170), (4200, 4600, 405), (5250, 5700, 600)), fill_ln2=((125, 400, 530), (135, 450, 285)),
    fill_attn=((5440, 6900, 9050, 0.5, 325), (8350, 12300, 15900, 0.5, 375)),
    wqkv=((1040, 1440), (1870, 2520), (3400, 4200)), wo=(7300, 9250), w1=(9500, 13600), w2=(13850, 16850),
    nested=(16500, 18550), late_copies=(4000, 7400), mod=(3740, 5700, 7600, 9500, 15500),
    tail_attn=((40, 2055, 4250, 0.41, 330), (170, 1885, 3750, 0.5, 275)), tail_ln2=((150, 600, 300), (165, 500, 380)),
)


class Schedule:
    def __init__(self):
        self.issued = 0.0
        self.now = 0.0
        self.count = 0
        self.tasks, self.due, self.results = [], [], []

    def add(self, when, task):
        heapq.heappush(self.tasks, (when, self.count, task))
        self.count += 1

    def spread(self, tasks, t0, t1):
        for i, task in enumerate(tasks):
            self.add(self.issued + t0 + (t1 - t0) * i / len(tasks), task)

    def run_until(self, t):
        while self.tasks and self.tasks[0][0] < t:
            self.now, _, task = heapq.heappop(self.tasks)
            step = next(task, None)
            if step is not None:
                self.add(self.now + step, task)

    def run_next(self):
        self.run_until(self.tasks[0][0] + 1e-3)

    def drain(self):
        self.run_until(np.inf)
        self.due, self.results = [], []

    def record(self, result, cost):
        self.results.append((self.issued, cost, result))
        self.issued += cost

    def tick(self, lead):
        t = self.now - lead
        for t0, cost, r in self.results:
            if t0 <= t < t0 + cost:
                row = 8 * int((t - t0) / cost * (r.shape[0] // 8))
                return r[row:row + 8, 0:128]
        return None


def call(fn, *args):
    fn(*args)
    yield


def run(gen):
    for _ in gen:
        pass


def dot(a, b):
    return jnp.dot(a, b, preferred_element_type=f32)


def total(parts):
    return functools.reduce(jnp.add, parts)


def tile_rows(v, n):
    return v if n == 8 else jnp.concatenate([v] * (n // 8), axis=0)


def bits(x):
    return x if x.dtype == i32 else pltpu.bitcast(x, i32)


def load_bf16(ref, row, n):
    words = ref if ref.dtype == i32 else ref.bitcast(i32)
    return pltpu.bitcast(words[row // 2:(row + n) // 2, :], bf16)


def across_tiles(ref, row):
    return ref.bitcast(i32)[pl.ds(row // 2, 8, stride=TILE_PITCH // 2 + 1), :]


def rsqrt(x):
    return jnp.exp2(jnp.log(x) * (-0.5 * LOG2E))


def barrel(xs, step):
    group = lax.broadcasted_iota(i32, (8, 128), 1) // H
    ys = [jnp.where(group % 2 == 1, xs[(i + step) % 4], xs[i]) for i in range(4)]
    return [jnp.where(group >= 2, ys[(i + 2) % 4], ys[i]) for i in range(4)]


def strassen_lhs(a11, a12, a21, a22):
    return [a11 + a22, a21 + a22, a11, a22, a11 + a12, a21 - a11, a12 - a22]


def strassen_rhs(b11, b12, b21, b22):
    return [b11 + b22, b11, b12 - b22, b21 - b11, b22, b11 + b12, b21 + b22]


def strassen_out(products, emit, bias=lambda half, v: v):
    m2 = next(products)
    m4 = bias(0, next(products))
    emit(1, 0, m2 + m4)
    yield
    m5 = next(products)
    c11 = m4 - m5
    m3 = bias(1, next(products))
    emit(0, 1, m3 + m5)
    yield
    c22 = m3 - m2
    m1 = next(products)
    c11, c22 = c11 + m1, c22 + m1
    emit(0, 0, c11 + next(products))
    yield
    emit(1, 1, c22 + next(products))


def block_kernel(x_hbm, wqkv_hbm, wo_hbm, w1_hbm, b1_hbm, w2_hbm, b2_hbm, c_hbm, wmod_hbm, out_hbm,
                 x_v, wqkv_v, wo_v, w1_v, b1_v, w2_v, b2_v, c_v, wmod_v, out_v, in_sems, out_sems,
                 wo_wide, w1_nested, y_s, y_nested, qk_s, v_s, h_s, x1_s, o_s, act_s, wqkv_s, sums_s):
    sums_s = dict(zip((0, 1, 2, 'wo', 'w1', 'w2'), sums_s))
    sched = Schedule()
    fixed = {}
    val = {}
    ready = set()
    holder = {}
    riders = []
    dma = {}
    counts = dict(copies=3, waits=0)
    small = [pltpu.make_async_copy(src, dst, in_sems.at[i])
             for i, (src, dst) in enumerate(((c_hbm, c_v), (b1_hbm, b1_v), (b2_hbm, b2_v)))]

    def fence(ref, lead, row, always=False):
        x = sched.tick(lead)
        if x is None and always:
            x = fixed['zero']
        if x is not None:
            x = x if x.dtype == ref.dtype else pltpu.bitcast(x, ref.dtype)
            ref[pl.ds(pl.multiple_of(fixed['offset'] + row, 8), 8), :] = x

    def finish_by(when, *deps):
        sched.due.append((when, functools.reduce(jnp.bitwise_or, [bits(d) for d in deps])))

    def finish(*deps):
        finish_by(sched.now, *deps)

    def wait_for_due(cols, cost):
        counts['waits'] += 1
        cols = list(cols)
        col = cols[counts['waits'] % len(cols)]
        rows, later = {}, []
        for when, dep in sched.due:
            if when < sched.issued + cost:
                row = 8 * int(max(when - sched.issued, 0.0) / cost * (col.shape[0] // 8))
                rows[row] = dep if row not in rows else rows[row] | dep
            else:
                later.append((when, dep))
        sched.due = later
        parts, r = [], 0
        for row in sorted(rows):
            dep = rows[row] if col.dtype == i32 else pltpu.bitcast(rows[row], col.dtype)
            parts += [col[r:row], jnp.where(fixed['zero'] == 0, col[row:row + 8], dep)]
            r = row + 8
        parts.append(col[r:])
        cols[counts['waits'] % len(cols)] = jnp.concatenate([p for p in parts if p.shape[0]], axis=0)
        return cols

    def request(name, src, dst, row, blocks):
        sem, ends = in_sems.at[counts['copies']], [row]
        counts['copies'] += 1
        for r, n, b in blocks:
            pltpu.make_async_copy(
                src.at[r:r + n, b * 128:(b + 1) * 128], dst.at[ends[-1]:ends[-1] + n, :], sem).start()
            ends.append(ends[-1] + n)
        dma[name] = dst, ends, sem

    def request_x(j0, j1):
        request(('x', j0), x_hbm.at[0], x_v, j0 * NB * T, [(j * T, T, b) for j in range(j0, j1) for b in range(NB)])

    def request_mod(j):
        request(('mod', j), wmod_hbm, wmod_v, j * NB * D, [(0, D, j * NB + b) for b in range(NB)])

    def request_early():
        small[0].start()
        request_x(0, 1)
        request_mod(1)
        for kh in range(2):
            request(('wq', kh), wqkv_hbm, wqkv_v, kh * NB * D // 2, [(kh * D // 2, D // 2, b) for b in range(NB)])
        request_x(1, 2)
        for p in (1, 2):
            request(('wqkv', p), wqkv_hbm, wqkv_v, p * NB * D, [(0, D, p * NB + b) for b in range(NB)])
        request_mod(0)
        request_x(2, 3)
        request_x(NT - 1, NT)
        request_mod(2)
        request('wo', wo_hbm, wo_v, 0, [(0, D, b) for b in range(NB)])
        request_mod(4)
        request_mod(3)

    def request_w1():
        for cp in small[1:]:
            cp.start()
        for _, _, n0, n1 in UP:
            request(('w1', n0), w1_hbm, w1_v, 2 * n0 * D, [(0, D, h + n) for n in range(n0, n1) for h in (0, FH)])

    def request_rest():
        for k0, k1 in ((0, 4), (4, FH)):
            request(('w2', k0), w2_hbm, w2_v, 2 * NB * k0 * 128,
                    [((h + k0) * 128, (k1 - k0) * 128, b) for h in (0, FH) for b in range(NB)])
        request_mod(5)
        request_x(3, NT - 1)

    def arrive(name, after=None):
        if name not in dma:
            return
        dst, ends, sem = dma.pop(name)
        words = dst.bitcast(i32)
        after = sched.tick(150) if after is None else after
        if after is not None:
            spare = words.shape[0] - 8
            words[pl.ds(pl.multiple_of(fixed['offset'] + spare, 8), 8), :] = bits(after)
            finish_by(sched.now + 60, words[spare:spare + 8, :])
        filled = dst.at[ends[0]:ends[-1], :]
        pltpu.make_async_copy(filled, filled, sem).wait()
        finish_by(sched.now + 60, *[words[end // 2 - 8:end // 2, :] for end in ends[1:]])

    class Tile:
        def __init__(self, base, off, qkv=0, h=0, x1=0, o=0):
            self.base, self.off, self.slot = base, off, qkv
            self.qk, self.v = qk_s[qkv], v_s[qkv]
            self.h, self.x1, self.o = h_s[h], x1_s[x1], o_s[o]
            index = base + off if isinstance(base, int) else None
            self.nested = index not in (0, NT - 2)
            self.first, self.last = index == 0, index == NT - 1
            self.unshifted = index in (0, 1)

        def rows(self, r, n):
            start = self.base * T + (self.off * T + r)
            return pl.ds(start if isinstance(start, int) else pl.multiple_of(start, TH), n)

        def x(self, b, r, n):
            start = self.base * (NB * TH) + ((self.off * NB + b) * T + r) // 2
            start = start if isinstance(start, int) else pl.multiple_of(start, 8)
            return pltpu.bitcast(x_v.bitcast(i32)[pl.ds(start, n // 2), :], bf16).astype(f32)

        def out_copy(self):
            rows = self.rows(0, T)
            return pltpu.make_async_copy(out_v.at[rows, :], out_hbm.at[0, rows, :], out_sems.at[self.base + self.off])

        def out_block_copy(self, h, hn):
            rows, cols = self.rows(h * TH, TH), pl.ds(hn * D // 2, D // 2)
            return pltpu.make_async_copy(out_v.at[rows, cols], out_hbm.at[0, rows, cols], out_sems.at[NT + 2 * h + hn])

    def seg(b):
        return b * PITCH + 8 + HALO

    def row_times(key, row, column, post=lambda r: r):
        cols = []

        def step(b):
            cols.append(dot(tile_rows(fixed[row], 16).astype(bf16), column(b))[:8])
            sched.issued += 16
            if b == NB - 1:
                fixed[key] = post(jnp.concatenate(cols, axis=1))
        riders.extend(functools.partial(step, b) for b in range(NB))

    def fetch_mod(j, after=None):
        arrive(('mod', j), after)
        post = {1: lambda r: r + 1.0, 4: lambda r: r + 1.0, 5: lambda r: r * (0.5 / ALPHA),
                3: lambda r: r - jnp.mean(r, axis=1, keepdims=True)}.get(j, lambda r: r)
        row_times(('mod', j), 'cond', lambda b: load_bf16(wmod_v, (j * NB + b) * D, D), post)

    def fetch_shift():
        fetch_mod(0)
        for p in range(3):
            assert ('permuted', p) in ready
            row_times(('shift', p), ('mod', 0), functools.partial(lambda p, b: jnp.concatenate(
                [weight_tile(p, k // 2, b // 2, k % 2, b % 2) for k in range(NB)], axis=0), p))

    def vector(key, b, n=8):
        while key not in fixed:
            riders.pop(0)()
        return tile_rows(fixed[key][:, b * 128:(b + 1) * 128], n)

    def permute_wqkv(p, quadrants):
        arrive(('wqkv', p))
        lane = lax.broadcasted_iota(i32, (D // 4, 128), 1)
        dl, hb, hl, quad = lane // H, lane % H // 8, lane % 8, lane % DH // 4
        for kh, nh in quadrants:
            src = [wqkv_v.bitcast(i32)[pl.ds((2 * (p * NB + b) + kh if p else kh * NB + b) * D // 4, D // 4), :]
                   for b in range(NB)]
            pair = [jnp.where(quad % 2 == 1, src[(i + 1 - nh) % 4], src[(i - nh) % 4]) for i in (0, 2)]
            for n in range(2):
                wqkv_s[4 * p + 2 * kh + nh][pl.ds(n * D // 4, D // 4), :] = jnp.take_along_axis(
                    jnp.where(quad >= 2, pair[1 - n], pair[n]), hl * DH + (hb + nh + 2 * n) % 4 * 4 + dl,
                    axis=1, mode='promise_in_bounds')
        ready.add(('permuted', p))

    def widen_wo(u0, u1):
        arrive('wo')
        fence(wo_v.bitcast(i32), TIMING['weight_lead'], NB * D // 2)
        for u in range(u0, u1):
            wo_wide[pl.ds(u * HEAD_PITCH, DH), :] = (
                load_bf16(wo_v, u * DH, DH).astype(f32) * vector(('mod', 2), u // H, DH))
        finish(wo_wide[pl.ds(u0 * HEAD_PITCH, 8, stride=HEAD_PITCH), :])

    def weight_tile(name, kh, nh, k, n, r=0, rows=128):
        if name == 'wo':
            turn, n = kh + 2 * k, 2 * nh + n
            return jnp.concatenate(
                [wo_wide[pl.ds((n * H + hb * 8) * HEAD_PITCH + 4 * ((hb + turn) % 4) + dl, 8, stride=HEAD_PITCH), :]
                 for dl, hb in (divmod(u // 8, 4) for u in range(r, r + rows, 8))], axis=0)
        if name == 'w1':
            return load_bf16(w1_v, (2 * n + nh) * D + (2 * kh + k) * 128 + r, rows)
        if name == 'w2':
            k0, k1 = (0, 4) if k < 4 else (4, FH)
            return load_bf16(w2_v, (2 * NB * k0 + (kh * NB + 2 * nh + n) * (k1 - k0) + k - k0) * 128 + r, rows)
        return load_bf16(wqkv_s[4 * name + 2 * kh + nh], n * D // 2 + k * 128 + r, rows)

    def built(name):
        return tuple(range(7)) if name == 'wo' else SUMS

    def operand_row(name, i, k, n):
        return ((2 * k + n if name == 'w2' else 2 * n + k) * len(built(name)) + built(name).index(i)) * TILE_PITCH

    def build_operands(name, pair, r):
        if name == 'wo':
            fence(wo_wide, TIMING['weight_lead'], NB * H * HEAD_PITCH, True)
        elif name in ('w1', 'w2'):
            arrive((name, pair))
            fence((w1_v if name == 'w1' else w2_v).bitcast(i32), TIMING['weight_lead'], FH * D)
        else:
            assert ('permuted', name) in ready
            for u in range(4):
                fence(wqkv_s[4 * name + u], TIMING['weight_lead'], D // 2, True)
        ref = sums_s[name]
        tiles = [(pair, j) if name == 'w2' else (j, pair) for j in range(2)]
        for k, n in tiles:
            ops = strassen_rhs(*[weight_tile(name, kh, nh, k, n, r, 16).astype(f32)
                                 for kh in range(2) for nh in range(2)])
            for i in built(name):
                row = operand_row(name, i, k, n) + r
                ref[row:row + 16, :] = ops[i].astype(bf16)
            if r == 112:
                ready.add((name, k, n))
        row = operand_row(name, 0, *tiles[0]) + r
        count = len(built(name))
        for j in range(2):
            finish(*[ref.bitcast(i32)[pl.ds((row + u * TILE_PITCH) // 2, 8), :] for u in range(j * count, (j + 1) * count)])

    def prepare(name, pairs, t0, t1):
        tasks = [call(widen_wo, u, u + 8) for u in range(0, NB * H, 8)] if name == 'wo' else []
        tasks += [call(build_operands, name, p, r) for p in range(pairs) for r in range(0, 128, 16)]
        sched.spread(tasks, t0, t1)

    def operand(name, i, k, n, r=0, rows=128):
        plain = i not in built(name)
        if name == 'w2':
            arrive((name, k - k % 4))
        while (name, k, n) not in ready and not (plain and (name == 'w2' or ('permuted', name) in ready)):
            sched.run_next()
        if plain:
            return weight_tile(name, i // 4, i // 4, k, n, r, rows)
        return load_bf16(sums_s[name], operand_row(name, i, k, n) + r, rows)

    def nested_row(n0, i, j):
        return ((n0 // 2 * 7 + i) * len(SUMS) + SUMS.index(j)) * 128

    def build_nested(n0, i0, r):
        fence(sums_s['w1'].bitcast(i32), TIMING['weight_lead'], FH * len(SUMS) * TILE_PITCH)
        fence(w1_v.bitcast(i32), TIMING['weight_lead'], FH * D)
        for i in range(i0, min(i0 + 2, 7)):
            ops = strassen_rhs(*[operand('w1', i, k, n, r, 16).astype(f32) for k in range(2) for n in (n0, n0 + 1)])
            for j in SUMS:
                w1_nested[nested_row(n0, i, j) + r:nested_row(n0, i, j) + r + 16, :] = ops[j].astype(bf16)
            finish(*[w1_nested.bitcast(i32)[pl.ds((nested_row(n0, i, j) + r) // 2, 8), :] for j in SUMS])

    def rowsum(parts):
        s = total(parts)
        finish(s[-8:])
        return jnp.sum(s, axis=1, keepdims=True)

    def collect(name, ref, r, parts, nested=False):
        assert holder.setdefault(id(ref), name) == name
        n = parts[0].shape[0] // 2
        seen = val.setdefault((name, r // 16), [])
        seen.append([p[:n] for p in parts] + [p[n:] for p in parts])
        if (r + n) % 16:
            finish(*seen[-1])
            return
        r -= r % 16
        cols = [jnp.concatenate([p[b] for p in seen], axis=0) for b in range(2 * NB)]
        ops = [strassen_lhs(*cols[k::2]) for k in range(2)]
        for k in range(2):
            for i in range(7):
                ref[pl.ds((k * 7 + i) * TILE_PITCH + r, 16), :] = ops[k][i].astype(bf16)
        if nested and r < TH // 2:
            val['top', name, r] = ops
        elif nested:
            q = r - TH // 2
            top = val['top', name, q]
            for i in range(7):
                for j, op in enumerate(strassen_lhs(top[0][i], top[1][i], ops[0][i], ops[1][i])):
                    y_nested[pl.ds((7 * i + j) * NESTED_PITCH + q, 16), :] = op.astype(bf16)
            finish(*[y_nested.bitcast(i32)[pl.ds((u * NESTED_PITCH + q) // 2, 8, stride=NESTED_PITCH // 2 + 1), :]
                     for u in (0, 8, 16, 24, 32, 40, 41)])
        ready.add((name, r))
        finish(*[across_tiles(ref, u * TILE_PITCH + r) for u in (0, 6)])

    def complete(name):
        while not all((name, r) in ready for r in range(0, TH, 16)):
            sched.run_next()

    def stored_lhs(name, ref):
        def get(i, k0, k1, cost):
            complete(name)
            cols = [ref.bitcast(i32)[pl.ds((k * 7 + i) * TILE_PITCH // 2, TH // 2), :] for k in range(k0, k1)]
            return jnp.concatenate([pltpu.bitcast(c, bf16) for c in wait_for_due(cols, cost)], axis=1)
        return get

    def first_rows(b, h):
        return jnp.concatenate([val['normed', r][b][16 * h:16 * h + 16] for r in range(0, TH, 16)],
                               axis=0) * vector(('mod', 1), b, TH)

    def first_lhs(i, k0, k1, cost):
        if ('first', i) not in val:
            val['first', i] = [strassen_lhs(*[first_rows(b, h) for h in range(2) for b in (k, 2 + k)])[i]
                               for k in range(k0, k1)]
        return jnp.concatenate(wait_for_due(val['first', i], cost), axis=1).astype(bf16)

    def ln1_chunk(t, r, lag):
        arrive(('x', t.off))
        xs = [jnp.concatenate([t.x(b, h + r, 16) for h in (0, TH)], axis=0) for b in range(NB)]
        mean = rowsum(xs)
        yield lag
        mean = mean * (1.0 / D)
        ds = [x - mean for x in xs]
        var = rowsum([d * d for d in ds])
        yield lag + 30
        rs = rsqrt(var * (1.0 / D) + EPS)
        hs = [d * rs for d in ds]
        if t.first:
            val['normed', r] = hs
            return
        hs = [hs[b] * vector(('mod', 1), b, 32) for b in range(NB)]
        if not t.unshifted:
            hs = [hs[b] + vector(('mod', 0), b, 32) for b in range(NB)]
        collect(('h', t.off), t.h, r, hs)

    def ln2_chunk(t, r, lag):
        assert ('x1', t.off) in ready
        xs = [jnp.concatenate([t.x1[b * T + h + r:b * T + h + r + 8, :] for h in (0, TH)], axis=0) for b in range(NB)]
        mean = rowsum(xs)
        yield lag
        mean = mean * (1.0 / D)
        ds = [x - mean for x in xs]
        es = [ds[b] * vector(('mod', 4), b, 16) for b in range(NB)]
        var, mean = rowsum([d * d for d in ds]), rowsum(es)
        yield lag + 30
        rs, mean = rsqrt(var * (1.0 / D) + EPS), mean * (1.0 / D)
        ds = [(es[b] - mean) * rs + vector(('mod', 3), b, 16) for b in range(NB)]
        var = rowsum([d * d for d in ds])
        yield lag + 30
        rs = rsqrt(var * (1.0 / (D * ALPHA * ALPHA)) + EPS / (ALPHA * ALPHA))
        collect(('y', t.off), y_s, r, [d * rs for d in ds], nested=t.nested)

    def attn_chunk(t, h, r, dt, lag):
        assert {('qkv', 0, t.off), ('qkv', 1, t.off)} <= ready
        r0 = h * TH + r
        masked = t.first and r0 < 2 * (W - 1)

        def key(b, w):
            k = t.qk[pl.ds(seg(b) + r0 - 2 * w, 8), :]
            return k + vector(('shift', 1), b) if masked else k

        parts = []
        for u in range(2):
            fence(t.qk, TIMING['key_lead'], 0)
            qs = [t.qk[pl.ds(seg(NB + b) + r0, 8), :] for b in range(NB)]
            if t.unshifted:
                qs = [qs[b] + vector(('shift', 0), b) for b in range(NB)]
            diag = barrel([total([qs[b] * key(b, w) for b in range(NB)]) for w in range(4 * u, 4 * u + 4)], 1)
            finish(diag[0])
            parts.append([diag[0]] + [pltpu.roll(diag[i], H * i, 1) for i in range(1, 4)])
            yield lag if u else 0.23 * dt
        logits = [total(p) * (DH ** -0.5 * LOG2E) for p in parts]
        if masked:
            pos = r0 + lax.broadcasted_iota(i32, (8, 128), 0)
            group = lax.broadcasted_iota(i32, (8, 128), 1) // H
            logits = [jnp.where(pos >= 2 * (4 * u + group), logits[u], -1e9 * LOG2E) for u in range(2)]
        peak = jnp.maximum(*logits)
        finish(peak)
        peaks = [peak] + [pltpu.roll(peak, H * i, 1) for i in range(1, 4)]
        yield lag + 16
        peak = functools.reduce(jnp.maximum, peaks)
        es = [jnp.exp2(x - peak) for x in logits]
        finish(es[1])
        es = [[e] + [pltpu.roll(e, 128 - H * i, 1) for i in range(1, 4)] for e in es]
        spent = 0.23 * dt + 2 * lag + 16
        yield (np.ceil((spent + lag) / dt - 0.5) + 0.5) * dt - spent
        assert ('qkv', 2, t.off) in ready
        inv = pl.reciprocal(total(es[0] + es[1]), full_range=False)
        es = barrel(es[0], -1) + barrel(es[1], -1)
        out = [total([es[w] * t.v[pl.ds(seg(b) + r0 - 2 * w, 8), :] for w in range(W)]) * inv for b in range(NB)]
        if t.unshifted:
            out = [out[b] + vector(('shift', 2), b) for b in range(NB)]
        if r0 == T - 8:
            holder.pop(t.slot)
        yield 0.46 * dt
        if h == 0:
            val['upper', t.off, r] = out
            finish(*out)
        else:
            collect(('o', t.off), t.o, r,
                    [jnp.concatenate([a, b], axis=0) for a, b in zip(val['upper', t.off, r], out)])

    def ln1(t, t0, t1, lag):
        sched.spread([ln1_chunk(t, r, lag) for r in range(0, TH, 16)], t0, t1)

    def ln2(t, t0, t1, lag):
        sched.spread([ln2_chunk(t, r + q + e, lag)
                      for r in range(0, TH // 2, 16) for q in (0, TH // 2) for e in (0, 8)], t0, t1)

    def attn(t, t0, t_mid, t1, share, lag):
        n = T // 8
        at = [np.interp(i / n, [0, share, 1], [t0, t_mid, t1]) for i in range(n + 1)]
        for i in range(n):
            sched.add(sched.issued + at[i], attn_chunk(t, i % 2, i // 2 * 8, at[i + 1] - at[i], lag))

    def rhs(tile, k0, k1, n0, n1):
        return jnp.concatenate(
            [jnp.concatenate([tile(k, n) for n in range(n0, n1)], axis=1) for k in range(k0, k1)], axis=0)

    def products(lhs, name, pieces, ahead=()):
        def issue(i, piece, split=False):
            k0, k1, n0, n1 = piece
            cost = (k1 - k0) * (n1 - n0) * TH / 4
            sched.run_until(sched.issued + cost)
            a, b = lhs(i, k0, k1, cost), rhs(functools.partial(operand, name, i), *piece)
            r = jnp.concatenate([dot(a[u:u + TH // 2], b) for u in (0, TH // 2)], axis=0) if split else dot(a, b)
            sched.record(r, cost)
            for _ in range(min(len(riders), 1 if ('shift', 0) in fixed else 2)):
                riders.pop(0)()
            return r

        whole = [p for p in pieces if (p[1] - p[0]) * (p[3] - p[2]) == 4]
        half = [p for p in pieces if p not in whole]
        order = ahead + tuple(i for i in ORDER if i not in ahead)
        groups = [order[u:u + 2] for u in range(0, 7, 2)] if half else [(i,) for i in order]
        done = {}
        for want in ORDER:
            while want not in done:
                group = groups.pop(0)
                for i in group:
                    done[i] = [issue(i, p) for p in whole]
                for i in group:
                    done[i] += [issue(i, p, len(group) == 1) for p in half]
            yield total(done[want])

    def nested_products(n0):
        def inner(i):
            for group in (ORDER[:4], ORDER[4:]):
                results = []
                for j in group:
                    sched.run_until(sched.issued + TH / 8)
                    a = y_nested.bitcast(i32)[pl.ds((7 * i + j) * NESTED_PITCH // 2, TH // 4), :]
                    (a,) = wait_for_due([a], TH / 8)
                    b = (load_bf16(w1_nested, nested_row(n0, i, j), 128) if j in SUMS
                         else operand('w1', i, j // 4, n0 + j // 4))
                    results.append(dot(pltpu.bitcast(a, bf16), b))
                    sched.record(results[-1], TH / 8)
                yield from results

        for i in ORDER:
            blocks = {}
            run(strassen_out(inner(i), lambda h, hn, v: blocks.update({(h, hn): v})))
            yield jnp.concatenate([jnp.concatenate([blocks[h, 0], blocks[h, 1]], axis=1) for h in range(2)], axis=0)

    def by_tile(emit, n0=0):
        def split(h, hn, v):
            for u in range(v.shape[1] // 128):
                emit(h, hn, n0 + u, v[:, u * 128:(u + 1) * 128])
        return split

    def biased(key, half, n0=0):
        return lambda hn, v: v + tile_rows(fixed[key][:, (hn * half + n0) * 128:][:, :v.shape[1]], TH)

    def first_q(t):
        out = [[], []]
        for kh in range(2):
            sched.now = sched.issued
            arrive(('wq', kh), sched.tick(TIMING['wq_lead']) if kh else vector(('mod', 1), 0))
            permute_wqkv(0, ((kh, 0), (kh, 1)))
            cols = [jnp.concatenate([first_rows(b, h) for h in range(2)], axis=0) for b in (2 * kh, 2 * kh + 1)]
            for nh in range(2):
                sched.run_until(sched.issued + T)
                a = jnp.concatenate(wait_for_due(cols, T), axis=1).astype(bf16)
                out[nh].append(dot(a, rhs(functools.partial(weight_tile, 0, kh, nh), *SQUARE)))
                sched.record(out[nh][-1], T)
        q = jnp.concatenate([total(o) for o in out], axis=1)
        for b in range(NB):
            t.qk[seg(NB + b):seg(NB + b) + T, :] = q[:, b * 128:(b + 1) * 128]
        ready.add(('qkv', 0, t.off))

    def copy_halo(t, prev, p):
        dst, src = (t.v, prev.v) if p == 2 else (t.qk, prev.qk)
        for b in range(NB):
            rows = src[seg(b) + T - HALO:seg(b) + T, :]
            if prev.unshifted and not t.unshifted:
                rows = rows + vector(('shift', p), b, HALO)
            dst[seg(b) - HALO:seg(b), :] = rows

    def qkv(t, prev, parts):
        for p in parts:
            dst, first_tile = (t.v, 0) if p == 2 else (t.qk, NB * (1 - p))

            def emit(h, hn, n, v):
                row = seg(first_tile + 2 * hn + n)
                dst[row + h * TH:row + (h + 1) * TH, :] = v
                if t.first and h == 0:
                    dst[row - HALO:row, :] = jnp.broadcast_to(v[0:1, :], (HALO, 128))

            sched.run_until(sched.issued + 1)
            assert holder.setdefault(t.slot, t.off) == t.off
            if p and prev:
                copy_halo(t, prev, p)
            stream = (products(first_lhs, p, [SQUARE], PLAIN) if t.first
                      else products(stored_lhs(('h', t.off), t.h), p, [SQUARE]))
            run(strassen_out(stream, by_tile(emit)))
            ready.add(('qkv', p, t.off))
            if p == 2:
                holder.pop(id(t.h), None)

    def proj(t):
        def emit(h, hn, n, v):
            row = (2 * hn + n) * T + h * TH
            t.x1[row:row + TH, :] = t.x(2 * hn + n, h * TH, TH) + v
            for r in (0, TH // 2):
                finish_by(sched.issued + TIMING['after_matmul'] + r - TH // 2, t.x1[pl.ds(row + r, 8, stride=9), :])
        run(strassen_out(products(stored_lhs(('o', t.off), t.o), 'wo', [SQUARE]), by_tile(emit)))
        fence(t.x1, np.inf, NB * T, True)
        ready.add(('x1', t.off))
        holder.pop(id(t.o))

    def up(t):
        def emit(h, hn, n, v):
            ref, row = act_s[n // 2], ((h * 2 + hn) * 2 + n % 2) * TH
            ref[row:row + TH, :] = v + v * jnp.tanh(v * (KAPPA + v * v))
            for r in (0, TH // 2):
                finish_by(sched.issued + TIMING['after_matmul'] + r + 32 * (n % 2) - TH + 32,
                          ref[pl.ds(row + r, 8, stride=9), :])
        complete(('y', t.off))
        for piece in UP:
            n0, n1 = piece[2:]
            stream = (nested_products(n0) if n1 - n0 == 2 and t.nested
                      else products(stored_lhs(('y', t.off), y_s), 'w1', [piece]))
            run(strassen_out(stream, by_tile(emit, n0), biased('b1', FH, n0)))
        holder.pop(id(y_s))

    def down(t):
        def emit(h, hn, n, v):
            b = 2 * hn + n
            y = t.x1[b * T + h * TH:b * T + (h + 1) * TH, :] + vector(('mod', 5), b, TH) * v
            out_v[t.rows(h * TH, TH), b * 128:(b + 1) * 128] = y.astype(out_v.dtype)
            if t.last and n == 1:
                t.out_block_copy(h, hn).start()

        def lhs(i, k0, k1, cost):
            sched.now = sched.issued
            ref = act_s[k0 // 2]
            fence(ref, TIMING['act_lead'], 8 * TH, True)
            cols = [strassen_lhs(*[ref[(u * 2 + k % 2) * TH:(u * 2 + k % 2 + 1) * TH, :] for u in range(4)])[i]
                    for k in range(k0, k1)]
            return jnp.concatenate(wait_for_due(cols, cost), axis=1).astype(bf16)
        return strassen_out(products(lhs, 'w2', DOWN, PLAIN if t.first else ()), by_tile(emit), biased('b2', 2))

    def resume(off):
        val.clear()
        ready.clear()
        ready.update((name, k, n) for name in sums_s for k in range(FH) for n in range(FH))
        ready.update((('y', off), r) for r in range(0, TH, 16))
        ready.update(('qkv', p, off + u) for p in range(3) for u in (1, 2)[:1 + (off > 0)])
        holder.clear()
        holder.update({id(y_s): ('y', off), 0: off + 1, 3: NT - 1})

    def scale_biases():
        for cp in small[1:]:
            cp.wait()
        fixed['b1'] = jnp.broadcast_to(b1_v[...].astype(f32).reshape(1, F) * ALPHA, (8, F))
        fixed['b2'] = jnp.broadcast_to(b2_v[...].astype(f32).reshape(1, D) * (2 * ALPHA), (8, D))

    request_early()
    small[0].wait()
    c = c_v[...].astype(f32)
    fixed['zero'] = bits(jnp.broadcast_to(c[:, 0:128], (8, 128))) & 0xFFFF
    fixed['offset'] = fixed['zero'][0, 0]
    fixed['cond'] = jnp.broadcast_to(c * jax.nn.sigmoid(c), (8, D))

    t0, t1, t2 = Tile(0, 0, qkv=1, x1=1), Tile(0, 1, qkv=2, h=1, o=1), Tile(0, 2)
    final = Tile(0, NT - 1, qkv=3, h=2)
    ln1(t0, 0, 100, 500)
    sched.run_until(np.inf)
    fetch_mod(1, val['normed', TH - 16][0][0:8])
    vector(('mod', 1), 0)
    for when, requests in zip(TIMING['late_copies'], (request_w1, request_rest)):
        sched.add(sched.issued + when, call(requests))
    for j, when in zip((0, 2, 4, 3, 5), TIMING['mod']):
        sched.add(sched.issued + when, call(fetch_mod, j) if j else call(fetch_shift))
    for p, when in enumerate(TIMING['wqkv']):
        if p:
            sched.add(sched.issued + when[0] - TIMING['permute_lead'],
                      call(permute_wqkv, p, ((0, 0), (1, 1), (1, 0), (0, 1))))
        prepare(p, 2, *when)
    for t, when in zip((t1, t2, final), TIMING['fill_ln1']):
        ln1(t, *when)
    for t, when in zip((t0, t1), TIMING['fill_attn']):
        attn(t, *when)
    prepare('wo', 2, *TIMING['wo'])
    prepare('w1', FH, *TIMING['w1'])
    prepare('w2', FH, *TIMING['w2'])
    sched.spread([call(build_nested, n0, i, r)
                  for n0 in (0, 2, 4) for i in (0, 2, 4, 6) for r in range(0, 128, 16)], *TIMING['nested'])
    first_q(t0)
    qkv(t1, t0, [0])
    for p in (1, 2):
        qkv(t0, None, [p])
        qkv(t1, t0, [p])
    qkv(t2, t1, [0, 1, 2])
    qkv(final, None, [0])
    proj(t0)
    ln2(t0, *TIMING['fill_ln2'][0])
    qkv(final, None, [1, 2])
    scale_biases()
    up(t0)
    rest = down(t0)
    next(rest)
    next(rest)
    proj(t1)
    ln2(t1, *TIMING['fill_ln2'][1])
    run(rest)
    sched.drain()
    arrive(('x', 3))
    sched.drain()
    assert not dma and not riders
    t0.out_copy().start()

    def steady(j, carry):
        resume(0)
        a, b, c = (Tile(j, off) for off in range(3))
        attn(b, *TIMING['attn'])
        ln1(c, *TIMING['ln1'])
        ln2(b, *TIMING['ln2'])
        up(a)
        run(down(a))
        proj(b)
        complete(('o', b.off))
        qkv(c, b, [0, 1, 2])
        sched.drain()
        a.out_copy().start()
        return carry
    lax.fori_loop(1, NT - 3, steady, 0)

    resume(NT - 3)
    tail = [Tile(0, NT - 3), Tile(0, NT - 2, x1=1), Tile(0, NT - 1, qkv=3)]
    for p in (1, 2):
        copy_halo(tail[2], tail[1], p)
    for a, b, attn_at, ln2_at in zip(tail, tail[1:], TIMING['tail_attn'], TIMING['tail_ln2']):
        attn(b, *attn_at)
        up(a)
        rest = down(a)
        next(rest)
        next(rest)
        proj(b)
        ln2(b, *ln2_at)
        run(rest)
    for t in tail[:2]:
        t.out_copy().start()
    up(tail[2])
    run(down(tail[2]))
    for j in range(NT - 1):
        Tile(0, j).out_copy().wait()
    for u in range(4):
        tail[2].out_block_copy(*divmod(u, 2)).wait()


@jax.jit
def pallas_adaLN_cond__sliding_local_dilated__mixer_channel_mlp__prompt_kernel(
        A_x, A_wqkv, A_wo, B_x, B_w1, B_b1, B_w2, B_b2, c, w_mod):
    del B_x
    hbm = pl.BlockSpec(memory_space=pltpu.HBM)

    def tiles(rows, dtype, spare=True):
        return pltpu.VMEM((rows + (32 // jnp.dtype(dtype).itemsize if spare else 0), 128), dtype)

    return pl.pallas_call(
        block_kernel,
        in_specs=[hbm] * 9,
        out_specs=hbm,
        out_shape=jax.ShapeDtypeStruct((1, S, D), A_x.dtype),
        scratch_shapes=[
            tiles(NB * S, bf16), tiles(3 * NB * D, bf16), tiles(NB * D, bf16), tiles(2 * FH * D, bf16),
            pltpu.VMEM((F,), bf16), tiles(NB * F, bf16), pltpu.VMEM((D,), bf16), pltpu.VMEM((1, D), bf16),
            tiles(6 * NB * D, bf16), pltpu.VMEM((S, D), bf16),
            pltpu.SemaphoreType.DMA((25,)), pltpu.SemaphoreType.DMA((NT + 4,)),
            tiles(NB * H * HEAD_PITCH, f32), tiles(21 * len(SUMS) * 128, bf16, False),
            tiles(14 * TILE_PITCH, bf16, False), tiles(49 * NESTED_PITCH, bf16, False),
            [tiles(2 * NB * PITCH, f32, False)] * 4, [tiles(NB * PITCH, f32, False)] * 4,
            [tiles(14 * TILE_PITCH, bf16, False)] * 3, [tiles(NB * T, f32)] * 2,
            [tiles(14 * TILE_PITCH, bf16, False)] * 2,
            [tiles(8 * TH, f32)] * 4, [tiles(D // 2, i32)] * 12,
            [tiles(28 * TILE_PITCH, bf16, False)] * 4 + [tiles(2 * FH * len(SUMS) * TILE_PITCH, bf16)] * 2,
        ],
        compiler_params=pltpu.CompilerParams(
            vmem_limit_bytes=96 * 1024 * 1024, flags={'XLA_TPU_RESCHEDULE_DMA_DONES': True},
            disable_bounds_checks=True, disable_semaphore_checks=True),
        name='fused_block',
    )(A_x, A_wqkv, A_wo, B_w1, B_b1, B_w2, B_b2, c, w_mod)
```
